```python
import os as _os
_os.environ.setdefault("JAX_PLATFORMS", "cpu")
import jax
import jax.numpy as jnp

def _softmax(x, axis=-1):
    return jax.nn.softmax(x, axis=axis)
def _gelu(x):
    return jax.nn.gelu(x, approximate=True)
def _silu(x):
    return jax.nn.silu(x)
def _sigmoid(x):
    return jax.nn.sigmoid(x)
def _layernorm(x, axis=-1, eps=1e-5):
    m = jnp.mean(x, axis=axis, keepdims=True)
    v = jnp.var(x, axis=axis, keepdims=True)
    return (x - m) / jnp.sqrt(v + eps)
def _scatter_add(tgt, idx, src, axis=0):
    return tgt.at[idx].add(src)
def _segment_sum(src, seg, n):
    return jax.ops.segment_sum(src, seg, n)
class _Rng:
    def __init__(self, key):
        self._k = key
    def _next(self):
        self._k, sub = jax.random.split(self._k)
        return sub
    def normal(self, shape):
        return jax.random.normal(self._next(), shape, dtype=jnp.bfloat16)
    def randint(self, lo, hi, shape):
        return jax.random.randint(self._next(), shape, lo, hi, dtype=jnp.int32)
    def uniform(self, shape, lo=0.0, hi=1.0):
        return jax.random.uniform(self._next(), shape, jnp.bfloat16, lo, hi)
    def permutation(self, n):
        return jax.random.permutation(self._next(), n)


kernel_name = 'gated_mix__spectral_gfnet__dense_activation_silu__prompt'

def setup_inputs():
    _rng = _Rng(jax.random.key(int.from_bytes(__import__("os").urandom(4), "little")))
    _w = (lambda a: (lambda t: t.astype(jnp.bfloat16) if jnp.issubdtype(t.dtype, jnp.floating) else t)(jnp.asarray(a)))
    def _A_setup():
        B, S, D = 1, 2048, 512
        Df = D // 2 + 1
        return {
            "x": _w((lambda *s: _rng.normal(s) * 0.05)(B, S, D)),
            "w_r": _w((lambda *s: _rng.normal(s) * 0.05)(S, Df) * 0.02),
            "w_i": _w((lambda *s: _rng.normal(s) * 0.05)(S, Df) * 0.02),
        }
    _A_in = _A_setup()

    def _B_setup():
        B, S, D, F = 1, 2048, 512, 1376
        return {
            "x": _w((lambda *s: _rng.normal(s) * 0.05)(B, S, D)),
            "w1": _w((lambda *s: _rng.normal(s) * 0.05)(D, F) * (D ** -0.5)),
            "w2": _w((lambda *s: _rng.normal(s) * 0.05)(F, D) * (F ** -0.5)),
        }
    _B_in = _B_setup()

    return {
        "A_x": _A_in["x"],
        "A_w_r": _A_in["w_r"],
        "A_w_i": _A_in["w_i"],
        "B_x": _B_in["x"],
        "B_w1": _B_in["w1"],
        "B_w2": _B_in["w2"],
        "gate_w": _w((lambda *s: _rng.normal(s) * 0.05)(512) * 16.0),
    }

def reference(A_x, A_w_r, A_w_i, B_x, B_w1, B_w2, gate_w):
    def _A_ref(x, w_r, w_i):
        B, S, D = x.shape
        X = (lambda x, axes=(-2,-1): jnp.fft.rfft2(x.astype(jnp.float32), axes=axes))(x, axes=(-2, -1))
        W = w_r + 1j * w_i
        X = X * W
        y = (lambda x, s, axes=(-2,-1): jnp.fft.irfft2(x, s=s, axes=axes).astype(jnp.bfloat16))(X, (S, D), axes=(-2, -1))
        return y

    def _B_ref(x, w1, w2):
        h = jnp.einsum("bsd,df->bsf", x, w1)
        h = _silu(h)
        out = jnp.einsum("bsf,fd->bsd", h, w2)
        return out

    x = A_x
    g = _sigmoid((x * gate_w).sum(-1, keepdims=True))
    a = _A_ref(x, A_w_r, A_w_i)
    b = _B_ref(x, B_w1, B_w2)
    return g * a + (1 - g) * b
```

```python
import numpy as np
import ml_dtypes
import jax
import jax.numpy as jnp
from jax import lax
import jax.experimental.pallas as pl
import jax.experimental.pallas.tpu as pltpu

S, D, F = 2048, 512, 1376
H = D // 2
N1, N2 = 128, 16
RB = 128
NB = S // RB
NB3 = 9
BF = ml_dtypes.bfloat16


def _consts():
    d = np.arange(D)[:, None].astype(np.float64)
    k = np.arange(H)[None, :].astype(np.float64)
    ang = 2 * np.pi * d * k / D
    alt = (-1.0) ** np.arange(D)
    fr, fi = np.cos(ang), -np.sin(ang)
    fi[:, 0] = alt
    fd = np.concatenate([fr, fi], axis=1)
    gr, gi = 2 * np.cos(ang).T, -2 * np.sin(ang).T
    gr[0, :] = 1.0
    gi[0, :] = alt
    gd = np.concatenate([gr, gi], axis=0) / D
    m = np.arange(64)
    ka = np.concatenate([4 * m, 4 * m + 2]); kb = ka + 1
    ca = np.concatenate([ka, H + ka]); cb = np.concatenate([kb, H + kb])
    m0 = np.tile(np.arange(128) < 64, 2)
    fd = np.concatenate([fd[:128, ca] * m0, fd[:128, ca] * ~m0, fd[:256, cb]], axis=0)
    gd = np.concatenate([np.concatenate([gd[ca, :128] * m0[:, None],
                                         gd[ca, :128] * ~m0[:, None]], axis=1),
                         gd[cb, :256]], axis=0)
    a = np.arange(N1).astype(np.float64)
    th = 2 * np.pi * np.outer(a, a) / N1
    c, s = np.cos(th), np.sin(th)
    f1 = np.block([[c, s], [-s, c]])
    g1 = np.block([[c, -s], [s, c]]) / S
    tw = 2 * np.pi * np.outer(np.arange(N1), np.arange(N2)) / S
    twc = np.zeros((N1, 128)); tws = np.zeros((N1, 128))
    twc[:, :N2] = np.cos(tw); tws[:, :N2] = np.sin(tw)
    f1s = np.concatenate([c, -s], axis=1)
    g1s = np.concatenate([c, -s], axis=0) / S
    b = np.arange(N2).astype(np.float64)
    t2 = 2 * np.pi * np.outer(b, b) / N2
    c2, s2 = np.cos(t2), np.sin(t2)
    f2 = np.block([[c2, s2], [-s2, c2]])
    g2 = np.block([[c2, -s2], [s2, c2]])
    tws_side = np.concatenate([np.cos(tw).T, np.sin(tw).T], axis=0)
    return dict(
        fd=fd.astype(BF), gd=gd.astype(BF), f1=f1.astype(BF), g1=g1.astype(BF),
        tw=np.concatenate([twc, tws], axis=0).astype(np.float32),
        f1s=f1s.astype(BF), g1s=g1s.astype(BF),
        f2=np.concatenate([f2, g2], axis=0).astype(BF),
        tws=tws_side.astype(np.float32))


_C = _consts()


def _fft16(xr, xi, sign):
    def fft4(r, i):
        ar, ai = r[0] + r[2], i[0] + i[2]
        br, bi = r[0] - r[2], i[0] - i[2]
        cr, ci = r[1] + r[3], i[1] + i[3]
        dr, di = r[1] - r[3], i[1] - i[3]
        if sign < 0:
            o1 = (br + di, bi - dr); o3 = (br - di, bi + dr)
        else:
            o1 = (br - di, bi + dr); o3 = (br + di, bi - dr)
        return [(ar + cr, ai + ci), o1, (ar - cr, ai - ci), o3]
    st = [fft4([xr[4 * n1 + n2] for n1 in range(4)],
               [xi[4 * n1 + n2] for n1 in range(4)]) for n2 in range(4)]
    outr, outi = [None] * 16, [None] * 16
    for k1 in range(4):
        r, i = [], []
        for n2 in range(4):
            vr, vi = st[n2][k1]
            m = (n2 * k1) % 16
            if m == 0:
                pass
            elif m == 4:
                vr, vi = (vi, -vr) if sign < 0 else (-vi, vr)
            elif m in (2, 6):
                h = np.float32(np.sqrt(0.5))
                p, q = (vr + vi) * h, (vi - vr) * h
                if sign > 0:
                    p, q = (vr - vi) * h, (vr + vi) * h
                if m == 6:
                    p, q = (q, -p) if sign < 0 else (-q, p)
                vr, vi = p, q
            else:
                cc = np.float32(np.cos(2 * np.pi * m / 16))
                ss = np.float32(sign * np.sin(2 * np.pi * m / 16))
                vr, vi = vr * cc - vi * ss, vr * ss + vi * cc
            r.append(vr); i.append(vi)
        o = fft4(r, i)
        for k2 in range(4):
            outr[k1 + 4 * k2], outi[k1 + 4 * k2] = o[k2]
    return outr, outi


def _dot(a, b):
    return jnp.dot(a, b, preferred_element_type=jnp.float32)


def _kernel(ax_h, wr_h, wi_h, w1_h, w2_h, gw_h,
            fd_h, gd_h, f1_h, g1_h, tw_h, f1s_h, g1s_h, f2_h, tws_h,
            out_h,
            ax, wr, wi, w1, w2, gw, fd, gd, f1, g1, tw, f1s, g1s, f2, tws,
            wtmp, wrn, win, ybuf, abuf, bbuf, obuf, sems, osems):
    bf16, f32 = jnp.bfloat16, jnp.float32
    pairs = [(fd_h, fd), (f1_h, f1), (tw_h, tw),
             (w1_h, w1), (w2_h, w2), (wr_h, wr), (wi_h, wi),
             (f1s_h, f1s), (g1s_h, g1s), (f2_h, f2), (tws_h, tws),
             (g1_h, g1), (gd_h, gd), (gw_h, gw)]
    cps = [pltpu.make_async_copy(s_, d_, sems.at[n]) for n, (s_, d_) in enumerate(pairs)]
    def axcp(j):
        r = pl.multiple_of(j * 256, 256)
        return pltpu.make_async_copy(ax_h.at[pl.ds(r, 256), :], ax.at[pl.ds(r, 256), :],
                                     osems.at[j])
    cps[0].start()
    for j in range(S // 256):
        axcp(j).start()
    cps[0].wait()

    lane = lax.broadcasted_iota(jnp.int32, (N1, 128), 1)
    def p0(j, _):
        r0 = pl.multiple_of(j * 256, 256)
        axcp(j).wait()

        @pl.when(j == 0)
        def _():
            for cp in cps[1:3] + cps[5:7]:
                cp.start()

        @pl.when(j == 4)
        def _():
            for cp in cps[3:5] + cps[7:]:
                cp.start()

        x = [ax[pl.ds(r0, 256), c * 128:(c + 1) * 128].astype(f32) for c in range(4)]
        e, o = x[0] + x[2], x[1] + x[3]
        xa = _dot(jnp.concatenate([e + o, e - o], axis=1).astype(bf16), fd[0:256, :])
        xb = _dot(jnp.concatenate([x[0] - x[2], x[1] - x[3]], axis=1).astype(bf16), fd[256:, :])
        abuf[0, pl.ds(r0, 256), :] = xa[:, :128]
        abuf[2, pl.ds(r0, 256), :] = xa[:, 128:]
        abuf[1, pl.ds(r0, 256), :] = xb[:, :128]
        abuf[3, pl.ds(r0, 256), :] = xb[:, 128:]
        return 0

    lax.fori_loop(0, S // 256, p0, 0)

    def p1(b, ucol):
        v = [abuf[c4, pl.ds(b, N1, stride=N2), :] for c4 in range(4)]
        sel = lane == b
        ucol = jnp.where(sel, v[2][:, 0:1], ucol)
        im0 = jnp.where(lane == 0, 0.0, v[2])
        rhs = jnp.concatenate([jnp.concatenate([v[0], v[1]], axis=1),
                               jnp.concatenate([im0, v[3]], axis=1)], axis=0)
        y = _dot(f1[...], rhs.astype(bf16))
        c = jnp.sum(jnp.where(sel, tw[0:N1, :], 0.0), axis=1, keepdims=True)
        s = jnp.sum(jnp.where(sel, tw[N1:, :], 0.0), axis=1, keepdims=True)
        yr, yi = y[:N1], y[N1:]
        ybuf[b, 0:N1, :] = yr * c + yi * s
        ybuf[b, N1:2 * N1, :] = yi * c - yr * s
        return ucol

    for cp in cps[1:3] + cps[5:7]:
        cp.wait()

    def p1x(i, ucol):
        c0 = pl.multiple_of(i * 512, 512)
        for n, (src, dst) in enumerate(((wr, wrn), (wi, win))):
            for t in range(4):
                cc = pl.multiple_of(c0 + t * 128, 128)
                q = n * 4 + t
                wtmp[q] = src[0:H, pl.ds(cc, 128)].astype(f32)
                wp = jnp.concatenate([wtmp[q, pl.ds(o, 64, stride=4), :] for o in (0, 2, 1, 3)], axis=0)
                dst[pl.ds(cc, 128), :] = wp.T.astype(bf16)
        for t in range(4):
            ucol = p1(4 * i + t, ucol)
        return ucol

    ucol = lax.fori_loop(0, N2 // 4, p1x, jnp.zeros((N1, 128), f32), unroll=4)

    for cp in cps[3:5] + cps[7:11]:
        cp.wait()

    def ffn(r0):
        h = lax.dot_general(ax[pl.ds(r0, RB), :], w1[...], (((1,), (1,)), ((), ())),
                            preferred_element_type=f32)
        hh = 0.5 * h
        act = hh + hh * jnp.tanh(hh)
        return _dot(act.astype(bf16), w2[...])

    bbuf[8 * RB:9 * RB, :] = ffn(8 * RB)
    u = ucol.T[0:N2, :]
    t = _dot(u.astype(bf16), f1s[...])
    tc, ts = tws[0:N2, :], tws[N2:, :]
    tr, ti = t[:, :128], t[:, 128:]
    t = jnp.concatenate([tr * tc + ti * ts, ti * tc - tr * ts], axis=0)
    xs = _dot(f2[0:32, :], t.astype(bf16))
    l0 = lane == 0
    def nyq(ref):
        row = ref[H:H + 1, :].astype(f32)
        return jnp.concatenate([row[:, kb * N1:(kb + 1) * N1] for kb in range(N2)], axis=0)
    nr, ni = nyq(wr), nyq(wi)
    xr_, xi_ = xs[:N2], xs[N2:]
    zz = jnp.concatenate([xr_ * nr - xi_ * ni, xr_ * ni + xi_ * nr], axis=0)
    q = _dot(f2[32:64, :], zz.astype(bf16))
    qr, qi = q[:N2], q[N2:]
    q = jnp.concatenate([qr * tc - qi * ts, qi * tc + qr * ts], axis=1)
    yn = _dot(q.astype(bf16), g1s[...])
    yn_t = jnp.concatenate([yn, jnp.zeros((128 - N2, 128), f32)], axis=0).T

    def p2(j, _):
        r0 = pl.multiple_of(j * 16, 16)
        rb = pl.multiple_of(j * RB, RB)
        xb = ax[pl.ds(rb, RB), :]
        acc = [None]
        fch = [(0, 384), (384, 768), (768, 1152), (1152, F)]

        def fpart(n):
            lo, hi = fch[n]
            hh = 0.5 * lax.dot_general(xb, w1[lo:hi, :], (((1,), (1,)), ((), ())),
                                       preferred_element_type=f32)
            o = _dot((hh + hh * jnp.tanh(hh)).astype(bf16), w2[lo:hi, :])
            acc[0] = o if acc[0] is None else acc[0] + o

        for c in range(2):
            ls = slice(c * 128, (c + 1) * 128)
            wrs = [wrn[pl.ds(kb * N1 + r0, 16), ls].astype(f32) for kb in range(N2)]
            wis = [win[pl.ds(kb * N1 + r0, 16), ls].astype(f32) for kb in range(N2)]
            for hf in range(2):
                fpart(2 * c + hf)
                rr = pl.multiple_of(r0 + 8 * hf, 8)
                xr = [ybuf[b, pl.ds(rr, 8), ls] for b in range(N2)]
                xi = [ybuf[b, pl.ds(N1 + rr, 8), ls] for b in range(N2)]
                xr, xi = _fft16(xr, xi, -1)
                zr, zi = [], []
                for kb in range(N2):
                    a_, b_ = wrs[kb][8 * hf:8 * hf + 8], wis[kb][8 * hf:8 * hf + 8]
                    zr.append(xr[kb] * a_ - xi[kb] * b_)
                    zi.append(xr[kb] * b_ + xi[kb] * a_)
                zr, zi = _fft16(zr, zi, +1)
                for b in range(N2):
                    ybuf[b, pl.ds(rr, 8), ls] = zr[b]
                    ybuf[b, pl.ds(N1 + rr, 8), ls] = zi[b]
        bbuf[pl.ds(rb, RB), :] = acc[0]
        return 0

    lax.fori_loop(0, 8, p2, 0, unroll=8)

    for cp in cps[11:]:
        cp.wait()

    def p3(b, _):
        sel = lane == b
        c = jnp.sum(jnp.where(sel, tw[0:N1, :], 0.0), axis=1, keepdims=True)
        s = jnp.sum(jnp.where(sel, tw[N1:, :], 0.0), axis=1, keepdims=True)
        zr, zi = ybuf[b, 0:N1, :], ybuf[b, N1:2 * N1, :]
        z = jnp.concatenate([zr * c - zi * s, zi * c + zr * s], axis=0)
        v = _dot(g1[...], z.astype(bf16))
        ny = jnp.sum(jnp.where(sel, yn_t, 0.0), axis=1, keepdims=True)
        im0 = jnp.where(lane == 0, ny, v[N1:, :128])
        va = _dot(jnp.concatenate([v[:N1, :128], im0], axis=1).astype(bf16), gd[0:256, :])
        vb = _dot(jnp.concatenate([v[:N1, 128:], v[N1:, 128:]], axis=1).astype(bf16), gd[256:, :])
        e, o = va[:, :128] + va[:, 128:], va[:, :128] - va[:, 128:]
        for c4, val in enumerate((e + vb[:, :128], o + vb[:, 128:], e - vb[:, :128], o - vb[:, 128:])):
            abuf[c4, pl.ds(b, N1, stride=N2), :] = val
        return 0

    lax.fori_loop(0, N2, p3, 0, unroll=16)

    def mix(r0, slot, bval):
        x = ax[pl.ds(r0, RB), :].astype(f32)
        z = jnp.sum(x * gw[...].astype(f32).reshape(1, D), axis=1, keepdims=True)
        g = 0.5 + 0.5 * jnp.tanh(0.5 * z)
        a = jnp.concatenate([abuf[c, pl.ds(r0, RB), :] for c in range(4)], axis=1)
        obuf[pl.ds(r0, RB), :] = (g * a + (1.0 - g) * bval).astype(bf16)
        pltpu.make_async_copy(obuf.at[pl.ds(r0, RB), :], out_h.at[pl.ds(r0, RB), :],
                              osems.at[slot]).start()

    def p4(j, _):
        r1 = pl.multiple_of((j + NB3) * RB, RB)
        mix(r1, j + NB3, ffn(r1))
        r0 = pl.multiple_of(j * RB, RB)
        mix(r0, j, bbuf[pl.ds(r0, RB), :])
        return 0

    for j in (7, 8):
        mix(j * RB, j, bbuf[j * RB:(j + 1) * RB, :])
    lax.fori_loop(0, NB - NB3, p4, 0, unroll=7)
    for j in range(NB):
        pltpu.make_async_copy(obuf.at[pl.ds(j * RB, RB), :], out_h.at[pl.ds(j * RB, RB), :],
                              osems.at[j]).wait()


@jax.jit
def pallas_gated_mix__spectral_gfnet__dense_activation_silu__prompt_kernel(
    A_x, A_w_r, A_w_i, B_x, B_w1, B_w2, gate_w,
):
    bf16, f32 = jnp.bfloat16, jnp.float32
    names = ["fd", "gd", "f1", "g1", "tw", "f1s", "g1s", "f2", "tws"]
    consts = [_C[n] for n in names]
    ins = [A_x.reshape(S, D), A_w_r.T, A_w_i.T, B_w1.T, B_w2,
           gate_w] + consts
    anyspec = pl.BlockSpec(memory_space=pl.ANY)
    scratch = [pltpu.VMEM(x.shape, x.dtype) for x in ins] + [
        pltpu.VMEM((8, H, 128), f32),
        pltpu.VMEM((S, H), bf16),
        pltpu.VMEM((S, H), bf16),
        pltpu.VMEM((N2, 2 * N1 + 8, H), f32),
        pltpu.VMEM((4, S, 128), f32),
        pltpu.VMEM((NB3 * RB, D), f32),
        pltpu.VMEM((S, D), bf16),
        pltpu.SemaphoreType.DMA((15,)),
        pltpu.SemaphoreType.DMA((NB,)),
    ]
    out = pl.pallas_call(
        _kernel,
        in_specs=[anyspec] * len(ins),
        out_specs=anyspec,
        out_shape=jax.ShapeDtypeStruct((S, D), bf16),
        scratch_shapes=scratch,
        compiler_params=pltpu.CompilerParams(vmem_limit_bytes=100 * 1024 * 1024),
    )(*ins)
    return out.reshape(1, S, D)
```
